```python
import os as _os
_os.environ.setdefault("JAX_PLATFORMS", "cpu")
import jax
import jax.numpy as jnp

def _softmax(x, axis=-1):
    return jax.nn.softmax(x, axis=axis)
def _gelu(x):
    return jax.nn.gelu(x, approximate=True)
def _silu(x):
    return jax.nn.silu(x)
def _sigmoid(x):
    return jax.nn.sigmoid(x)
def _layernorm(x, axis=-1, eps=1e-5):
    m = jnp.mean(x, axis=axis, keepdims=True)
    v = jnp.var(x, axis=axis, keepdims=True)
    return (x - m) / jnp.sqrt(v + eps)
def _scatter_add(tgt, idx, src, axis=0):
    return tgt.at[idx].add(src)
def _segment_sum(src, seg, n):
    return jax.ops.segment_sum(src, seg, n)
class _Rng:
    def __init__(self, key):
        self._k = key
    def _next(self):
        self._k, sub = jax.random.split(self._k)
        return sub
    def normal(self, shape):
        return jax.random.normal(self._next(), shape, dtype=jnp.bfloat16)
    def randint(self, lo, hi, shape):
        return jax.random.randint(self._next(), shape, lo, hi, dtype=jnp.int32)
    def uniform(self, shape, lo=0.0, hi=1.0):
        return jax.random.uniform(self._next(), shape, jnp.bfloat16, lo, hi)
    def permutation(self, n):
        return jax.random.permutation(self._next(), n)


kernel_name = 'standalone__mha_softmax__decode'

def setup_inputs():
    _rng = _Rng(jax.random.key(int.from_bytes(__import__("os").urandom(4), "little")))
    _w = (lambda a: (lambda t: t.astype(jnp.bfloat16) if jnp.issubdtype(t.dtype, jnp.floating) else t)(jnp.asarray(a)))
    B, H, Sq, Sk, D = 1, 32, 1, 8192, 128
    return {
        "q": _w((lambda *s: _rng.normal(s) * 0.8)(B, H, Sq, D)),
        "k": _w((lambda *s: _rng.normal(s) * 0.8)(B, H, Sk, D)),
        "v": _w((lambda *s: _rng.normal(s) * 0.05)(B, H, Sk, D)),
    }

def reference(q, k, v):
    scale = q.shape[-1] ** -0.5
    scores = jnp.einsum("bhqd,bhkd->bhqk", q, k) * scale
    p = _softmax(scores, axis=-1)
    return jnp.einsum("bhqk,bhkd->bhqd", p, v)
```

```python
import jax
import jax.numpy as jnp
from jax import lax
import jax.experimental.pallas as pl
import jax.experimental.pallas.tpu as pltpu

_HEADS_PER_GROUP = 16
_ROWS_PER_GROUP = 128
_ROWS_PER_DMA = 64
_RING = 4
_PRIORITY = (0, 1, 1, 1)
_NT = (((1,), (1,)), ((), ()))


@jax.jit
def pallas_standalone__mha_softmax__decode_kernel(
    q: jax.Array,
    k: jax.Array,
    v: jax.Array,
):
    B, H, Sq, D = q.shape
    Sk = k.shape[2]
    S, G, r, ring = _HEADS_PER_GROUP, _ROWS_PER_GROUP, _ROWS_PER_DMA, _RING
    assert B == 1 and Sq == 1 and H % S == 0 and Sk % G == 0
    scale = D ** -0.5
    nsw = H // S
    nc = Sk // G
    n = nsw * nc
    assert n % ring == 0
    lead = ring - 1

    def kernel(q_hbm, k_hbm, v_hbm, o_hbm, buf, s_scr, q_buf, q_f32, m_scr, o_buf, sems, io_sem):
        def start(src, i, slot):
            h0 = (i // nc) * S
            r0 = lax.rem(i, nc) * G
            x = 0
            for j in range(G // r):
                for h in range(S):
                    pltpu.make_async_copy(
                        src.at[h0 + h, pl.ds(pl.multiple_of(r0 + j * r, r), r)],
                        buf.at[slot, h, pl.ds(j * r, r)],
                        sems.at[slot],
                    ).start(priority=_PRIORITY[x % len(_PRIORITY)])
                    x += 1

        def wait(slot):
            pltpu.make_async_copy(buf.at[slot], buf.at[slot], sems.at[slot]).wait()

        q_copy = pltpu.make_async_copy(q_hbm, q_buf, io_sem)
        q_copy.start()

        def prologue(i, _):
            start(k_hbm, i, i)

        lax.fori_loop(0, lead, prologue, None)

        q_copy.wait()
        q_f32[...] = q_buf[...].astype(jnp.float32)
        m_scr[...] = jnp.full(m_scr.shape, -jnp.inf, jnp.float32)

        row_g = lax.broadcasted_iota(jnp.int32, (8, G), 0)
        row_d = lax.broadcasted_iota(jnp.int32, (8, D), 0)

        def qk(i):
            slot = lax.rem(i, ring)
            wait(slot)
            h0 = (i // nc) * S
            r0 = pl.multiple_of(lax.rem(i, nc) * G, G)
            for b in range(S // 8):
                hs = pl.ds(pl.multiple_of(h0 + 8 * b, 8), 8)
                qs = q_f32[hs, :].astype(jnp.bfloat16)
                s = None
                for h in range(8):
                    sh = lax.dot_general(
                        qs, buf[slot, 8 * b + h], _NT, preferred_element_type=jnp.float32)
                    s = sh if s is None else jnp.where(row_g == h, sh, s)
                s = s * scale
                s_scr[hs, pl.ds(r0, G)] = s
                m = m_scr[hs, :]
                for c in range(G // 128):
                    m = jnp.maximum(m, s[:, c * 128:(c + 1) * 128])
                m_scr[hs, :] = m

        def body_k(i, _):
            start(k_hbm, i + lead, lax.rem(i + lead, ring))
            qk(i)

        lax.fori_loop(0, n - lead, body_k, None)

        def body_kv(i, _):
            start(v_hbm, i + lead - n, lax.rem(i + lead, ring))
            qk(i)

        lax.fori_loop(n - lead, n, body_kv, None)

        m_scr[...] = jnp.broadcast_to(jnp.max(m_scr[...], axis=-1, keepdims=True), m_scr.shape)

        for sw in range(nsw):
            def pv(i, carry, last=False):
                slot = lax.rem(i, ring)
                r0 = pl.multiple_of(lax.rem(i, nc) * G, G)
                ps, ls = [], []
                for b in range(S // 8):
                    hs = pl.ds(sw * S + 8 * b, 8)
                    m = m_scr[hs, :]
                    l = carry[b][0]
                    pp = []
                    for c in range(G // 128):
                        cols = pl.ds(pl.multiple_of(r0 + c * 128, 128), 128)
                        p = jnp.exp(s_scr[hs, cols] - m)
                        l = l + p
                        pp.append(p)
                    ps.append(jnp.concatenate(pp, axis=1).astype(jnp.bfloat16))
                    if last:
                        l = 1.0 / jnp.sum(l, axis=-1, keepdims=True)
                        l = jnp.broadcast_to(l, (8, D))
                    ls.append(l)
                wait(slot)
                out = []
                for b in range(S // 8):
                    o = None
                    for h in range(8):
                        oh = jnp.dot(
                            ps[b], buf[slot, 8 * b + h], preferred_element_type=jnp.float32)
                        o = oh if o is None else jnp.where(row_d == h, oh, o)
                    out.append((ls[b], carry[b][1] + o))
                return tuple(out)

            def body_v(i, carry):
                start(v_hbm, i + lead, lax.rem(i + lead, ring))
                return pv(i, carry)

            z = jnp.zeros((8, D), jnp.float32)
            carry = tuple((z, z) for _ in range(S // 8))
            lo, hi = sw * nc, (sw + 1) * nc
            if sw < nsw - 1:
                carry = lax.fori_loop(lo, hi - 1, body_v, carry)
                start(v_hbm, hi - 1 + lead, (hi - 1 + lead) % ring)
            else:
                carry = lax.fori_loop(lo, hi - lead, body_v, carry)
                carry = lax.fori_loop(hi - lead, hi - 1, pv, carry)
            carry = pv(hi - 1, carry, last=True)
            o = jnp.concatenate([a * li for (li, a) in carry], axis=0)
            o_buf[pl.ds(sw * S, S), :] = o.astype(o_buf.dtype)

        o_copy = pltpu.make_async_copy(o_buf, o_hbm, io_sem)
        o_copy.start()
        o_copy.wait()

    out = pl.pallas_call(
        kernel,
        in_specs=[pl.BlockSpec(memory_space=pltpu.HBM)] * 3,
        out_specs=pl.BlockSpec(memory_space=pltpu.HBM),
        out_shape=jax.ShapeDtypeStruct((H, D), q.dtype),
        scratch_shapes=[
            pltpu.VMEM((ring, S, G, D), k.dtype),
            pltpu.VMEM((H, Sk), jnp.float32),
            pltpu.VMEM((H, D), q.dtype),
            pltpu.VMEM((H, D), jnp.float32),
            pltpu.VMEM((H, 128), jnp.float32),
            pltpu.VMEM((H, D), q.dtype),
            pltpu.SemaphoreType.DMA((ring,)),
            pltpu.SemaphoreType.DMA(()),
        ],
        compiler_params=pltpu.CompilerParams(disable_bounds_checks=True),
    )(q.reshape(H, D), k.reshape(H, Sk, D), v.reshape(H, Sk, D))
    return out.reshape(q.shape)
```

```python
import jax
import jax.numpy as jnp
from jax import lax
import jax.experimental.pallas as pl
import jax.experimental.pallas.tpu as pltpu

_HEADS = 16
_KEYS = 128
_DMA_ROWS = 64
_RING = 4
_PRIORITY = (0, 1, 1, 1)
_TAIL_STAGES = (512, 384, 256, 128)
_SUB = 8
_NT = (((1,), (1,)), ((), ()))


def _aligned(x, n):
    return x if isinstance(x, int) else pl.multiple_of(x, n)


def _attention_kernel(
    q_hbm, k_hbm, v_hbm, o_hbm,
    ring, tail_v, tail_p, scores, row_max, q_in, q_f32, o_buf,
    ring_sems, tail_sems, io_sems,
):
    num_heads, num_keys, dim = k_hbm.shape
    scale = dim ** -0.5
    tiles = num_keys // _KEYS
    sets = num_heads // _HEADS
    groups = sets * tiles
    lead = _RING - 1
    tail_keys = sum(_TAIL_STAGES)
    shift = tiles.bit_length() - 1
    blocks = _HEADS // _SUB
    row = lax.broadcasted_iota(jnp.int32, (_SUB, dim), 0)

    def start(src, g, heads=_HEADS, ramp_up=False):
        slot = g & (_RING - 1)
        head0 = (g >> shift) * _HEADS
        key0 = (g & (tiles - 1)) * _KEYS
        for base in range(0, _KEYS, _DMA_ROWS):
            pieces = 2 if ramp_up and base == 0 else 1
            rows = _DMA_ROWS // pieces
            for h in range(heads):
                for u in range(pieces):
                    off = base + u * rows
                    pltpu.make_async_copy(
                        src.at[head0 + h, pl.ds(_aligned(key0 + off, rows), rows)],
                        ring.at[slot, h, pl.ds(off, rows)],
                        ring_sems.at[slot],
                    ).start(priority=_PRIORITY[(h * pieces + u) % len(_PRIORITY)])

    def wait(g, heads=_HEADS):
        slot = g & (_RING - 1)
        filled = ring.at[slot, pl.ds(0, heads)]
        pltpu.make_async_copy(filled, filled, ring_sems.at[slot]).wait()
        return slot

    q_copy = pltpu.make_async_copy(q_hbm, q_in, io_sems.at[0])
    q_copy.start()
    start(k_hbm, 0, ramp_up=True)
    lax.fori_loop(1, lead, lambda g, _: start(k_hbm, g), None)
    q_copy.wait()
    q_f32[...] = q_in[...].astype(jnp.float32)
    row_max[...] = jnp.full(row_max.shape, -jnp.inf, jnp.float32)

    def score_group(g):
        slot = wait(g)
        keys = pl.ds(_aligned((g & (tiles - 1)) * _KEYS, _KEYS), _KEYS)
        for b in range(blocks):
            hs = pl.ds(_aligned((g >> shift) * _HEADS + b * _SUB, _SUB), _SUB)
            q = q_f32[hs, :].astype(q_in.dtype)
            s = None
            for h in range(_SUB):
                s_h = lax.dot_general(
                    q, ring[slot, b * _SUB + h], _NT,
                    preferred_element_type=jnp.float32)
                s = s_h if s is None else jnp.where(row == h, s_h, s)
            s = s * scale
            scores[hs, keys] = s
            row_max[hs, :] = jnp.maximum(row_max[hs, :], s)

    def k_step(g, _):
        start(k_hbm, g + lead)
        score_group(g)

    def kv_step(g, _):
        start(v_hbm, g + lead - groups)
        score_group(g)

    lax.fori_loop(0, groups - lead, k_step, None)
    lax.fori_loop(groups - lead, groups, kv_step, None)
    row_max[...] = jnp.broadcast_to(
        jnp.max(row_max[...], axis=-1, keepdims=True), row_max.shape)

    def weights(head0, g, b):
        hs = pl.ds(head0 + b * _SUB, _SUB)
        keys = pl.ds(_aligned((g & (tiles - 1)) * _KEYS, _KEYS), _KEYS)
        return jnp.exp(scores[hs, keys] - row_max[hs, :])

    def accumulate(head0, lo, hi, carry, done=_HEADS, fetch=_HEADS):
        def step(g, carry):
            if fetch:
                start(v_hbm, g + lead, fetch)
            p = [weights(head0, g, b) for b in range(blocks)]
            slot = wait(g, done)
            out = []
            for b, (denom, acc) in enumerate(carry):
                p_b = p[b].astype(ring.dtype)
                o = jnp.zeros_like(acc)
                for h in range(min(_SUB, done - b * _SUB)):
                    o_h = jnp.dot(
                        p_b, ring[slot, b * _SUB + h],
                        preferred_element_type=jnp.float32)
                    o = jnp.where(row == h, o_h, o)
                out.append((denom + p[b], acc + o))
            return tuple(out)

        return lax.fori_loop(lo, hi, step, carry)

    zero = jnp.zeros((_SUB, dim), jnp.float32)
    init = ((zero, zero),) * blocks
    for i in range(sets - 1):
        carry = accumulate(i * _HEADS, i * tiles, (i + 1) * tiles, init)
        out = [acc / jnp.sum(denom, axis=-1, keepdims=True) for denom, acc in carry]
        o_buf[pl.ds(i * _HEADS, _HEADS), :] = jnp.concatenate(out).astype(o_buf.dtype)

    head0 = num_heads - _HEADS
    cut = groups - tail_keys // _KEYS
    carry = accumulate(head0, groups - tiles, cut - lead, init)
    carry = accumulate(head0, cut - lead, cut, carry, fetch=_HEADS - 1)
    carry = accumulate(head0, cut, groups - lead, carry, _HEADS - 1, _HEADS - 1)

    stages, first = [], 0
    for i, count in enumerate(_TAIL_STAGES):
        for off in range(first, first + count, _DMA_ROWS):
            pltpu.make_async_copy(
                v_hbm.at[num_heads - 1, pl.ds(num_keys - tail_keys + off, _DMA_ROWS)],
                tail_v.at[pl.ds(off, _DMA_ROWS)],
                tail_sems.at[i],
            ).start(priority=1)
        stages.append(pl.ds(first, count))
        first += count

    inv = []
    for b, (denom, _) in enumerate(carry):
        for g in range(groups - lead, groups):
            denom = denom + weights(head0, g, b)
        inv.append(jnp.broadcast_to(
            1.0 / jnp.sum(denom, axis=-1, keepdims=True), (_SUB, dim)))
    for g in range(cut, groups):
        p = weights(head0, g, blocks - 1) * inv[-1]
        tail_p[pl.ds((g - cut) * _KEYS, _KEYS), :] = jnp.broadcast_to(
            p[_SUB - 1:, :], (dim, _KEYS)).T

    carry = accumulate(head0, groups - lead, groups, carry, _HEADS - 1, 0)
    out = [acc * r for (_, acc), r in zip(carry, inv)]

    o_head = pltpu.make_async_copy(
        o_buf.at[pl.ds(0, head0)], o_hbm.at[pl.ds(0, head0)], io_sems.at[1])
    o_last = pltpu.make_async_copy(
        o_buf.at[pl.ds(head0, _HEADS)], o_hbm.at[pl.ds(head0, _HEADS)], io_sems.at[0])

    partial = jnp.where(row == _SUB - 1, out[-1], 0.0)
    for i, keys in enumerate(stages):
        if i == len(stages) - 1:
            o_head.start()
        filled = tail_v.at[keys]
        pltpu.make_async_copy(filled, filled, tail_sems.at[i]).wait()
        terms = tail_p[keys, :] * tail_v[keys, :].astype(jnp.float32)
        terms = [terms[j:j + _SUB] for j in range(0, keys.size, _SUB)]
        sums = [partial] + terms[:3]
        for j, term in enumerate(terms[3:]):
            sums[(j + 3) % 4] = sums[(j + 3) % 4] + term
        partial = (sums[0] + sums[1]) + (sums[2] + sums[3])
    out[-1] = jnp.where(
        row == _SUB - 1, jnp.sum(partial, axis=0, keepdims=True), out[-1])

    o_buf[pl.ds(head0, _HEADS), :] = jnp.concatenate(out).astype(o_buf.dtype)
    o_last.start()
    o_head.wait()
    o_last.wait()


@jax.jit
def pallas_standalone__mha_softmax__decode_kernel(
    q: jax.Array,
    k: jax.Array,
    v: jax.Array,
):
    batch, heads, q_len, dim = q.shape
    num_keys = k.shape[2]
    num_heads = batch * heads
    tiles = num_keys // _KEYS
    tail_keys = sum(_TAIL_STAGES)
    assert q_len == 1 and dim == _KEYS
    assert num_heads % _HEADS == 0 and num_heads > _HEADS
    assert num_keys % _KEYS == 0 and tiles & (tiles - 1) == 0
    assert tiles % _RING == 0 and num_keys >= tail_keys + _RING * _KEYS

    hbm = pl.BlockSpec(memory_space=pltpu.HBM)
    out = pl.pallas_call(
        _attention_kernel,
        in_specs=[hbm, hbm, hbm],
        out_specs=hbm,
        out_shape=jax.ShapeDtypeStruct((num_heads, dim), q.dtype),
        scratch_shapes=[
            pltpu.VMEM((_RING, _HEADS, _KEYS, dim), k.dtype),
            pltpu.VMEM((tail_keys, dim), v.dtype),
            pltpu.VMEM((tail_keys, dim), jnp.float32),
            pltpu.VMEM((num_heads, num_keys), jnp.float32),
            pltpu.VMEM((num_heads, _KEYS), jnp.float32),
            pltpu.VMEM((num_heads, dim), q.dtype),
            pltpu.VMEM((num_heads, dim), jnp.float32),
            pltpu.VMEM((num_heads, dim), q.dtype),
            pltpu.SemaphoreType.DMA((_RING,)),
            pltpu.SemaphoreType.DMA((len(_TAIL_STAGES),)),
            pltpu.SemaphoreType.DMA((2,)),
        ],
        compiler_params=pltpu.CompilerParams(disable_semaphore_checks=True),
    )(
        q.reshape(num_heads, dim),
        k.reshape(num_heads, num_keys, dim),
        v.reshape(num_heads, num_keys, dim),
    )
    return out.reshape(q.shape)
```
